```python
import os as _os
_os.environ.setdefault("JAX_PLATFORMS", "cpu")
import jax
import jax.numpy as jnp

def _softmax(x, axis=-1):
    return jax.nn.softmax(x, axis=axis)
def _gelu(x):
    return jax.nn.gelu(x, approximate=True)
def _silu(x):
    return jax.nn.silu(x)
def _sigmoid(x):
    return jax.nn.sigmoid(x)
def _layernorm(x, axis=-1, eps=1e-5):
    m = jnp.mean(x, axis=axis, keepdims=True)
    v = jnp.var(x, axis=axis, keepdims=True)
    return (x - m) / jnp.sqrt(v + eps)
def _scatter_add(tgt, idx, src, axis=0):
    return tgt.at[idx].add(src)
def _segment_sum(src, seg, n):
    return jax.ops.segment_sum(src, seg, n)
class _Rng:
    def __init__(self, key):
        self._k = key
    def _next(self):
        self._k, sub = jax.random.split(self._k)
        return sub
    def normal(self, shape):
        return jax.random.normal(self._next(), shape, dtype=jnp.bfloat16)
    def randint(self, lo, hi, shape):
        return jax.random.randint(self._next(), shape, lo, hi, dtype=jnp.int32)
    def uniform(self, shape, lo=0.0, hi=1.0):
        return jax.random.uniform(self._next(), shape, jnp.bfloat16, lo, hi)
    def permutation(self, n):
        return jax.random.permutation(self._next(), n)


kernel_name = 'standalone__gqa_softmax__near_ridge'

def setup_inputs():
    _rng = _Rng(jax.random.key(int.from_bytes(__import__("os").urandom(4), "little")))
    _w = (lambda a: (lambda t: t.astype(jnp.bfloat16) if jnp.issubdtype(t.dtype, jnp.floating) else t)(jnp.asarray(a)))
    B, Hq, Hkv, Sq, Sk, D = 8, 16, 8, 512, 512, 256
    return {
        "q": _w((lambda *s: _rng.normal(s) * 0.4)(B, Hq, Sq, D)),
        "k": _w((lambda *s: _rng.normal(s) * 0.4)(B, Hkv, Sk, D)),
        "v": _w((lambda *s: _rng.normal(s) * 0.05)(B, Hkv, Sk, D)),
    }

def reference(q, k, v):
    B, Hq, Sq, D = q.shape
    Hkv = k.shape[1]
    rep = Hq // Hkv
    k = jnp.repeat(k, rep, axis=1)
    v = jnp.repeat(v, rep, axis=1)
    scale = D ** -0.5
    scores = jnp.einsum("bhqd,bhkd->bhqk", q, k) * scale
    p = _softmax(scores, axis=-1)
    return jnp.einsum("bhqk,bhkd->bhqd", p, v)
```

```python
import math

import jax
import jax.numpy as jnp
from jax import lax
import jax.experimental.pallas as pl
import jax.experimental.pallas.tpu as pltpu


@jax.jit
def pallas_standalone__gqa_softmax__near_ridge_kernel(
    q: jax.Array,
    k: jax.Array,
    v: jax.Array,
):
    B, Hq, Sq, D = q.shape
    Hkv, Sk = k.shape[1], k.shape[2]
    rep = Hq // Hkv
    G = B * Hkv
    M = rep * Sq
    c = (D ** -0.5) * math.log2(math.e)

    def kernel_function(q_ref, k_ref, v_ref, o_ref):
        s = lax.dot_general(q_ref[...], k_ref[...], (((1,), (1,)), ((), ())),
                            preferred_element_type=jnp.float32)
        m = jnp.max(s, axis=-1, keepdims=True)
        p = jnp.exp2((s - m) * c)
        l = jnp.sum(p, axis=-1, keepdims=True)
        o = jnp.dot(p.astype(v_ref.dtype), v_ref[...], preferred_element_type=jnp.float32)
        o_ref[...] = (o * (1.0 / l)).astype(o_ref.dtype)

    out = pl.pallas_call(
        kernel_function,
        grid=(G,),
        in_specs=[pl.BlockSpec((None, M, D), lambda g: (g, 0, 0)),
                  pl.BlockSpec((None, Sk, D), lambda g: (g, 0, 0)),
                  pl.BlockSpec((None, Sk, D), lambda g: (g, 0, 0))],
        out_specs=pl.BlockSpec((None, M, D), lambda g: (g, 0, 0)),
        out_shape=jax.ShapeDtypeStruct((G, M, D), q.dtype),
        compiler_params=pltpu.CompilerParams(
            dimension_semantics=("parallel",), vmem_limit_bytes=64 << 20),
    )(q.reshape(G, M, D), k.reshape(G, Sk, D), v.reshape(G, Sk, D))
    return out.reshape(B, Hq, Sq, D)
```

```python
import math

import jax
import jax.numpy as jnp
from jax import lax
import jax.experimental.pallas as pl
import jax.experimental.pallas.tpu as pltpu

_BQ = 128
_LOOKAHEAD = 2
_SLOTS = 2
_MAX_UNROLL = 16
_FIRST_Q_CUTS = (1, 2, 3, 5)
_LAST_O_CUTS = (-3, -1)


@jax.jit
def pallas_standalone__gqa_softmax__near_ridge_kernel(
    q: jax.Array,
    k: jax.Array,
    v: jax.Array,
):
    B, Hq, Sq, D = q.shape
    Hkv, Sk = k.shape[1], k.shape[2]
    G = B * Hkv
    M = (Hq // Hkv) * Sq
    n_chunks = M // _BQ
    unroll = math.gcd(G, _MAX_UNROLL)
    n_iters = G // unroll
    assert M % _BQ == 0 and unroll % _SLOTS == 0 and n_chunks > _LOOKAHEAD
    exp2_scale = D**-0.5 * math.log2(math.e)
    q_cuts = [0, *(c for c in _FIRST_Q_CUTS if c < n_chunks), n_chunks]
    o_cuts = [0, *(n_chunks + c for c in _LAST_O_CUTS if n_chunks + c > 0), n_chunks]

    def kernel_function(q_hbm, k_hbm, v_hbm, o_hbm, kq_buf, v_buf, o_buf, in_sem, out_sem):
        def k_copy(g, slot):
            return pltpu.make_async_copy(
                k_hbm.at[g], kq_buf.at[slot, pl.ds(0, Sk)], in_sem.at[slot])

        def q_copy(g, slot):
            return pltpu.make_async_copy(
                q_hbm.at[g], kq_buf.at[slot, pl.ds(Sk, M)], in_sem.at[slot])

        def v_copy(g, slot):
            return pltpu.make_async_copy(
                v_hbm.at[g], v_buf.at[slot], in_sem.at[_SLOTS + slot])

        def o_copy(g, slot):
            return pltpu.make_async_copy(o_buf.at[slot], o_hbm.at[g], out_sem.at[slot])

        def first_q_piece(j):
            start, size = q_cuts[j] * _BQ, (q_cuts[j + 1] - q_cuts[j]) * _BQ
            return pltpu.make_async_copy(
                q_hbm.at[0, pl.ds(start, size)],
                kq_buf.at[0, pl.ds(Sk + start, size)],
                in_sem.at[2 * _SLOTS + j - 1 if j else 0],
            )

        def last_o_piece(j):
            rows = pl.ds(o_cuts[j] * _BQ, (o_cuts[j + 1] - o_cuts[j]) * _BQ)
            return pltpu.make_async_copy(
                o_buf.at[_SLOTS - 1, rows], o_hbm.at[G - 1, rows], out_sem.at[_SLOTS - 1])

        k_copy(0, 0).start()
        early = [j for j in range(len(q_cuts) - 1) if q_cuts[j] <= _LOOKAHEAD]
        for j in early:
            first_q_piece(j).start()
        v_copy(0, 0).start()
        for j in range(len(early), len(q_cuts) - 1):
            first_q_piece(j).start()
        for slot in range(1, _SLOTS):
            k_copy(slot, slot).start()
            q_copy(slot, slot).start()
            v_copy(slot, slot).start()

        def body(it, carry):
            def unless_first_iter(always, fn):
                fn() if always else pl.when(it > 0)(fn)

            def unless_last_iter(always, fn):
                fn() if always else pl.when(it < n_iters - 1)(fn)

            def probabilities(t):
                u, i = divmod(t, n_chunks)
                g, slot = it * unroll + u, u % _SLOTS
                if i == 0:
                    def wait_kq():
                        k_copy(g, slot).wait()
                        q_copy(g, slot).wait()

                    unless_first_iter(u > 0, wait_kq)
                    if u == 0:
                        pl.when(it == 0)(lambda: k_copy(0, 0).wait())
                if u == 0 and i in q_cuts:
                    pl.when(it == 0)(lambda: first_q_piece(q_cuts.index(i)).wait())

                s = lax.dot_general(
                    kq_buf[slot, pl.ds(Sk + i * _BQ, _BQ), :],
                    kq_buf[slot, pl.ds(0, Sk), :],
                    (((1,), (1,)), ((), ())),
                    preferred_element_type=jnp.float32,
                )

                if i == n_chunks - 1:
                    def refill_kq():
                        k_copy(g + _SLOTS, slot).start()
                        q_copy(g + _SLOTS, slot).start()

                    unless_last_iter(u + _SLOTS < unroll, refill_kq)

                m = jnp.max(s, axis=-1, keepdims=True)
                p = jnp.exp2((s - m) * exp2_scale)
                l = jnp.sum(p, axis=-1, keepdims=True)
                p = p * pltpu.reciprocal(l, approx=False, full_range=False)
                return p.astype(v_buf.dtype)

            def attend(t, p):
                u, i = divmod(t, n_chunks)
                g, slot = it * unroll + u, u % _SLOTS
                if i == 0:
                    v_copy(g, slot).wait()
                    unless_first_iter(u >= _SLOTS, lambda: o_copy(g - _SLOTS, slot).wait())

                o = jnp.dot(p, v_buf[slot], preferred_element_type=jnp.float32)
                o_buf[slot, pl.ds(i * _BQ, _BQ), :] = o.astype(o_buf.dtype)

                if u == unroll - 1 and i + 1 in o_cuts:
                    pl.when(it == n_iters - 1)(
                        lambda: last_o_piece(o_cuts.index(i + 1) - 1).start())
                if i == n_chunks - 1:
                    unless_last_iter(u < unroll - 1, lambda: o_copy(g, slot).start())
                    unless_last_iter(
                        u + _SLOTS < unroll, lambda: v_copy(g + _SLOTS, slot).start())

            total = unroll * n_chunks
            ready = {}
            for t in range(total + _LOOKAHEAD):
                if t < total:
                    ready[t] = probabilities(t)
                if t >= _LOOKAHEAD:
                    attend(t - _LOOKAHEAD, ready.pop(t - _LOOKAHEAD))
            return carry

        lax.fori_loop(0, n_iters, body, 0)

        for slot in range(_SLOTS - 1):
            o_copy(G - _SLOTS + slot, slot).wait()
        for j in range(len(o_cuts) - 1):
            last_o_piece(j).wait()

    out = pl.pallas_call(
        kernel_function,
        in_specs=[pl.BlockSpec(memory_space=pl.ANY)] * 3,
        out_specs=pl.BlockSpec(memory_space=pl.ANY),
        out_shape=jax.ShapeDtypeStruct((G, M, D), q.dtype),
        scratch_shapes=[
            pltpu.VMEM((_SLOTS, Sk + M, D), q.dtype),
            pltpu.VMEM((_SLOTS, Sk, D), v.dtype),
            pltpu.VMEM((_SLOTS, M, D), q.dtype),
            pltpu.SemaphoreType.DMA((2 * _SLOTS + len(q_cuts) - 2,)),
            pltpu.SemaphoreType.DMA((_SLOTS,)),
        ],
        compiler_params=pltpu.CompilerParams(
            vmem_limit_bytes=32 << 20,
            flags={"XLA_TPU_RESCHEDULE_DMA_DONES": True},
        ),
    )(q.reshape(G, M, D), k.reshape(G, Sk, D), v.reshape(G, Sk, D))
    return out.reshape(B, Hq, Sq, D)
```
